```python
import os as _os
_os.environ.setdefault("JAX_PLATFORMS", "cpu")
import jax
import jax.numpy as jnp

def _softmax(x, axis=-1):
    return jax.nn.softmax(x, axis=axis)
def _gelu(x):
    return jax.nn.gelu(x, approximate=True)
def _silu(x):
    return jax.nn.silu(x)
def _sigmoid(x):
    return jax.nn.sigmoid(x)
def _layernorm(x, axis=-1, eps=1e-5):
    m = jnp.mean(x, axis=axis, keepdims=True)
    v = jnp.var(x, axis=axis, keepdims=True)
    return (x - m) / jnp.sqrt(v + eps)
def _scatter_add(tgt, idx, src, axis=0):
    return tgt.at[idx].add(src)
def _segment_sum(src, seg, n):
    return jax.ops.segment_sum(src, seg, n)
class _Rng:
    def __init__(self, key):
        self._k = key
    def _next(self):
        self._k, sub = jax.random.split(self._k)
        return sub
    def normal(self, shape):
        return jax.random.normal(self._next(), shape, dtype=jnp.bfloat16)
    def randint(self, lo, hi, shape):
        return jax.random.randint(self._next(), shape, lo, hi, dtype=jnp.int32)
    def uniform(self, shape, lo=0.0, hi=1.0):
        return jax.random.uniform(self._next(), shape, jnp.bfloat16, lo, hi)
    def permutation(self, n):
        return jax.random.permutation(self._next(), n)


kernel_name = 'standalone__mha_softmax__sampling'

def setup_inputs():
    _rng = _Rng(jax.random.key(int.from_bytes(__import__("os").urandom(4), "little")))
    _w = (lambda a: (lambda t: t.astype(jnp.bfloat16) if jnp.issubdtype(t.dtype, jnp.floating) else t)(jnp.asarray(a)))
    B, H, Sq, Sk, D = 8, 32, 32, 2048, 128
    return {
        "q": _w((lambda *s: _rng.normal(s) * 0.4)(B, H, Sq, D)),
        "k": _w((lambda *s: _rng.normal(s) * 0.4)(B, H, Sk, D)),
        "v": _w((lambda *s: _rng.normal(s) * 0.05)(B, H, Sk, D)),
    }

def reference(q, k, v):
    scale = q.shape[-1] ** -0.5
    scores = jnp.einsum("bhqd,bhkd->bhqk", q, k) * scale
    p = _softmax(scores, axis=-1)
    return jnp.einsum("bhqk,bhkd->bhqd", p, v)
```

```python
import math

import jax
import jax.numpy as jnp
import jax.experimental.pallas as pl
import jax.experimental.pallas.tpu as pltpu

_GROUP = 4
_DEPTH = 3
_ROWS = 128


@jax.jit
def pallas_standalone__mha_softmax__sampling_kernel(
    q: jax.Array,
    k: jax.Array,
    v: jax.Array,
):
    B, H, Sq, D = q.shape
    Sk = k.shape[2]
    N = B * H
    G, depth, rows = _GROUP, _DEPTH, _ROWS
    n = N // G
    C = Sk // rows
    ahead = depth - 1
    assert N % G == 0 and Sk % rows == 0 and C % G == 0 and n > ahead
    exp2_scale = (D ** -0.5) * math.log2(math.e)

    def kernel(q_hbm, k_hbm, v_hbm, o_hbm, q_buf, kv_buf, o_buf, q_sem, kv_sem, o_sem):
        def start_q(g, slot):
            pltpu.make_async_copy(
                q_hbm.at[pl.ds(g * G, G)], q_buf.at[slot], q_sem.at[slot]
            ).start()

        def start_kv(g, slot, chunks):
            for c in chunks:
                for h in range(G):
                    for a, src in enumerate((k_hbm, v_hbm)):
                        pltpu.make_async_copy(
                            src.at[g * G + h, pl.ds(c * rows, rows)],
                            kv_buf.at[slot, a, h, pl.ds(c * rows, rows)],
                            kv_sem.at[slot],
                        ).start(priority=a)

        def wait_inputs(slot):
            pltpu.make_async_copy(q_buf.at[slot], q_buf.at[slot], q_sem.at[slot]).wait()
            pltpu.make_async_copy(kv_buf.at[slot], kv_buf.at[slot], kv_sem.at[slot]).wait()

        def head(g, slot, h):
            s = jax.lax.dot_general(
                q_buf[slot, h], kv_buf[slot, 0, h], (((1,), (1,)), ((), ())),
                preferred_element_type=jnp.float32,
            )
            m = jnp.max(s, axis=-1, keepdims=True)
            p = jnp.exp2((s - m) * exp2_scale)
            l = jnp.sum(p, axis=-1, keepdims=True)
            o = jnp.dot(
                p.astype(kv_buf.dtype), kv_buf[slot, 1, h],
                preferred_element_type=jnp.float32,
            )
            o_buf[g * G + h] = (o / l).astype(o_buf.dtype)

        def out_copy(h0):
            return pltpu.make_async_copy(
                o_buf.at[pl.ds(h0, G)], o_hbm.at[pl.ds(h0, G)], o_sem.at[0]
            )

        for d in range(ahead):
            start_q(d, d)
            start_kv(d, d, range(C))

        def steady(i, carry):
            slot = i % depth
            nslot = (i + ahead) % depth
            wait_inputs(slot)
            for h in range(G):
                if h == 0:
                    start_q(i + ahead, nslot)
                start_kv(i + ahead, nslot, range(h * C // G, (h + 1) * C // G))
                head(i, slot, h)
            return carry

        jax.lax.fori_loop(0, n - ahead, steady, None)

        def drain(i, carry):
            slot = i % depth
            wait_inputs(slot)
            for h in range(G):
                head(i, slot, h)
            return carry

        jax.lax.fori_loop(n - ahead, n - 1, drain, None)

        wait_inputs((n - 1) % depth)
        for j, h0 in enumerate(range(0, N - G, G)):
            out_copy(h0).start(priority=j % 2)
        for h in range(G):
            head(n - 1, (n - 1) % depth, h)
        out_copy(N - G).start()
        pltpu.make_async_copy(o_buf, o_buf, o_sem.at[0]).wait()

    out = pl.pallas_call(
        kernel,
        in_specs=[pl.BlockSpec(memory_space=pl.ANY)] * 3,
        out_specs=pl.BlockSpec(memory_space=pl.ANY),
        out_shape=jax.ShapeDtypeStruct((N, Sq, D), q.dtype),
        scratch_shapes=[
            pltpu.VMEM((depth, G, Sq, D), q.dtype),
            pltpu.VMEM((depth, 2, G, Sk, D), k.dtype),
            pltpu.VMEM((N, Sq, D), q.dtype),
            pltpu.SemaphoreType.DMA((depth,)),
            pltpu.SemaphoreType.DMA((depth,)),
            pltpu.SemaphoreType.DMA((1,)),
        ],
        compiler_params=pltpu.CompilerParams(vmem_limit_bytes=64 * 1024 * 1024),
    )(q.reshape(N, Sq, D), k.reshape(N, Sk, D), v.reshape(N, Sk, D))
    return out.reshape(B, H, Sq, D)
```

```python
import math

import numpy as np
import jax
import jax.numpy as jnp
import jax.experimental.pallas as pl
import jax.experimental.pallas.tpu as pltpu

_PIECE_BYTES = 32 * 1024
_Q_ORDER_BITS = (4, 5, 0, 1, 2, 3)
_OUT_ORDER_BITS = (2, 5, 4, 0, 1, 3)
_FINAL_ROUNDS = 2


def _piece_order(bits):
    return [
        sum(((i >> j) & 1) << bit for j, bit in enumerate(bits))
        for i in range(1 << len(bits))
    ]


def _loop(lo, hi, body):
    jax.lax.fori_loop(lo, hi, lambda i, carry: body(i), None)


@jax.jit
def pallas_standalone__mha_softmax__sampling_kernel(
    q: jax.Array,
    k: jax.Array,
    v: jax.Array,
):
    B, H, Sq, D = q.shape
    Sk = k.shape[2]
    rows = _PIECE_BYTES // (D * np.dtype(k.dtype).itemsize)
    heads = _PIECE_BYTES // (Sq * D * np.dtype(q.dtype).itemsize)
    rounds = Sk // rows
    half = B // 2
    pieces = H // heads
    assert rounds * rows == Sk and rounds == 2 * B and B == 2 * half
    assert pieces * heads == H and H >= 3
    q_order = [p for p in _piece_order(_Q_ORDER_BITS) if p < B * pieces]
    out_order = [p for p in _piece_order(_OUT_ORDER_BITS) if p < B * pieces]
    assert len(q_order) == len(out_order) == B * pieces
    exp2_scale = (D ** -0.5) * math.log2(math.e)

    def kernel(q_hbm, k_hbm, v_hbm, o_hbm, q_buf, kv_buf, o_buf, sems):
        last = H - 1
        last_slot = last % 2

        def fetch(h, batches, piece, sem):
            piece_rows = pl.ds(pl.multiple_of(piece * rows, rows), rows)
            for b in batches:
                for queue, src in enumerate((k_hbm, v_hbm)):
                    pltpu.make_async_copy(
                        src.at[b, h, piece_rows],
                        kv_buf.at[h % 2, queue, b, piece_rows],
                        sem,
                    ).start(priority=queue)

        def fetch_head(h, piece):
            fetch(h, range(B), piece, sems.at[h % 2])

        def fetch_last_head_first_half(step):
            for piece in (2 * step, 2 * step + 1):
                fetch(last, range(half), piece, sems.at[last_slot])

        def fetch_last_head_second_half(step):
            for piece in (2 * step, 2 * step + 1):
                final = piece >= rounds - _FINAL_ROUNDS
                sem = sems.at[jnp.where(final, 2, 1 - last_slot)]
                fetch(last, range(half, B), piece, sem)

        def wait_until_filled(buf, sem):
            pltpu.make_async_copy(buf, buf, sem).wait()

        def start_out(b, piece, queue):
            piece_heads = pl.ds(piece * heads, heads)
            pltpu.make_async_copy(
                o_buf.at[b, piece_heads], o_hbm.at[b, piece_heads], sems.at[last_slot]
            ).start(priority=queue)

        def attend(h, b):
            s = jax.lax.dot_general(
                q_buf[b, h],
                kv_buf[h % 2, 0, b],
                (((1,), (1,)), ((), ())),
                preferred_element_type=jnp.float32,
            )
            m = jnp.max(s, axis=-1, keepdims=True)
            p = jnp.exp2((s - m) * exp2_scale)
            l = jnp.sum(p, axis=-1, keepdims=True)
            o = jnp.dot(
                p.astype(kv_buf.dtype),
                kv_buf[h % 2, 1, b],
                preferred_element_type=jnp.float32,
            )
            o_buf[b, h] = (o / l).astype(o_buf.dtype)

        def process_head(h, fetch_during, fetch_after):
            wait_until_filled(kv_buf.at[h % 2], sems.at[h % 2])

            def step(b):
                attend(h, b)
                fetch_during(b)

            _loop(0, B, step)
            if fetch_after is not None:
                _loop(0, B, fetch_after)

        for i, p in enumerate(q_order):
            piece_heads = pl.ds((p % pieces) * heads, heads)
            pltpu.make_async_copy(
                q_hbm.at[p // pieces, piece_heads],
                q_buf.at[p // pieces, piece_heads],
                sems.at[2],
            ).start(priority=i % 2)
        _loop(0, rounds, lambda piece: fetch_head(0, piece))
        _loop(0, B, lambda piece: fetch_head(1, piece))
        wait_until_filled(q_buf, sems.at[2])

        _loop(
            0,
            H - 3,
            lambda h: process_head(
                h,
                lambda i: fetch_head(h + 1, B + i),
                lambda i: fetch_head(h + 2, i),
            ),
        )
        process_head(
            H - 3, lambda i: fetch_head(H - 2, B + i), fetch_last_head_first_half
        )
        process_head(H - 2, fetch_last_head_second_half, None)

        wait_until_filled(kv_buf.at[last_slot, :, pl.ds(0, half)], sems.at[last_slot])
        _loop(0, half, lambda b: attend(last, b))

        second_half = kv_buf.at[last_slot, :, pl.ds(half, half)]
        early_rows = (rounds - _FINAL_ROUNDS) * rows
        wait_until_filled(
            second_half.at[:, :, pl.ds(0, early_rows)], sems.at[1 - last_slot]
        )
        finished = [
            p for p in out_order if p // pieces < half or p % pieces < pieces - 1
        ]
        for i, p in enumerate(finished):
            start_out(p // pieces, p % pieces, i % 2)
        wait_until_filled(
            second_half.at[:, :, pl.ds(early_rows, Sk - early_rows)], sems.at[2]
        )

        def finish(b):
            attend(last, b)
            start_out(b, pieces - 1, 0)

        _loop(half, B, finish)
        wait_until_filled(o_buf, sems.at[last_slot])

    return pl.pallas_call(
        kernel,
        in_specs=[pl.BlockSpec(memory_space=pl.ANY)] * 3,
        out_specs=pl.BlockSpec(memory_space=pl.ANY),
        out_shape=jax.ShapeDtypeStruct(q.shape, q.dtype),
        scratch_shapes=[
            pltpu.VMEM(q.shape, q.dtype),
            pltpu.VMEM((2, 2, B, Sk, D), k.dtype),
            pltpu.VMEM(q.shape, q.dtype),
            pltpu.SemaphoreType.DMA((3,)),
        ],
        compiler_params=pltpu.CompilerParams(vmem_limit_bytes=48 * 1024 * 1024),
    )(q, k, v)
```

```python
import math

import numpy as np
import jax
import jax.numpy as jnp
import jax.experimental.pallas as pl
import jax.experimental.pallas.tpu as pltpu

_PIECE_BYTES = 32 * 1024
_Q_ORDER_BITS = (4, 5, 0, 1, 2, 3)
_OUT_ORDER_BITS = (2, 5, 4, 0, 1, 3)
_FINAL_PIECES = 11


def _piece_order(bits):
    return [
        sum(((i >> j) & 1) << bit for j, bit in enumerate(bits))
        for i in range(1 << len(bits))
    ]


def _loop(lo, hi, body):
    jax.lax.fori_loop(lo, hi, lambda i, carry: body(i), None)


@jax.jit
def pallas_standalone__mha_softmax__sampling_kernel(
    q: jax.Array,
    k: jax.Array,
    v: jax.Array,
):
    B, H, Sq, D = q.shape
    Sk = k.shape[2]
    rows = _PIECE_BYTES // (D * np.dtype(k.dtype).itemsize)
    heads = _PIECE_BYTES // (Sq * D * np.dtype(q.dtype).itemsize)
    rounds = Sk // rows
    half = B // 2
    pieces = H // heads
    before_final = rounds * half - _FINAL_PIECES
    assert rounds * rows == Sk and rounds == 2 * B and B == 2 * half
    assert pieces * heads == H and H >= 3 and heads >= 2 and before_final >= 0
    q_order = [p for p in _piece_order(_Q_ORDER_BITS) if p < B * pieces]
    out_order = [p for p in _piece_order(_OUT_ORDER_BITS) if p < B * pieces]
    assert len(q_order) == len(out_order) == B * pieces
    exp2_scale = (D ** -0.5) * math.log2(math.e)

    def kernel(q_hbm, k_hbm, v_hbm, o_hbm, q_buf, kv_buf, o_buf, sems):
        last = H - 1
        last_slot = last % 2

        def kv_copies(h, b, piece, sem):
            piece_rows = pl.ds(pl.multiple_of(piece * rows, rows), rows)
            return [
                pltpu.make_async_copy(
                    src.at[b, h, piece_rows], kv_buf.at[h % 2, i, b, piece_rows], sem
                )
                for i, src in enumerate((k_hbm, v_hbm))
            ]

        def start_kv(copies):
            for queue, copy in enumerate(copies):
                copy.start(priority=queue)

        def fetch_head(h, piece):
            for b in range(B):
                start_kv(kv_copies(h, b, piece, sems.at[h % 2]))

        def fetch_first_half(step):
            for piece in (2 * step, 2 * step + 1):
                for b in range(half):
                    start_kv(kv_copies(last, b, piece, sems.at[last_slot]))

        def fetch_second_half(step):
            for piece in (2 * step, 2 * step + 1):
                for j in range(half):
                    final = piece * half + j >= before_final
                    sem = sems.at[jnp.where(final, 2, 1 - last_slot)]
                    start_kv(kv_copies(last, half + j, piece, sem))

        def wait_second_half(i, sem):
            for copy in kv_copies(last, half + i % half, i // half, sem):
                copy.wait()

        def wait_until_filled(buf, sem):
            pltpu.make_async_copy(buf, buf, sem).wait()

        def start_out(batches, first_head, num_heads, queue):
            some_heads = pl.ds(first_head, num_heads)
            pltpu.make_async_copy(
                o_buf.at[batches, some_heads],
                o_hbm.at[batches, some_heads],
                sems.at[last_slot],
            ).start(priority=queue)

        def attend(h, b):
            s = jax.lax.dot_general(
                q_buf[b, h],
                kv_buf[h % 2, 0, b],
                (((1,), (1,)), ((), ())),
                preferred_element_type=jnp.float32,
            )
            m = jnp.max(s, axis=-1, keepdims=True)
            p = jnp.exp2((s - m) * exp2_scale)
            l = jnp.sum(p, axis=-1, keepdims=True)
            o = jnp.dot(
                p.astype(kv_buf.dtype),
                kv_buf[h % 2, 1, b],
                preferred_element_type=jnp.float32,
            )
            o_buf[b, h] = (o / l).astype(o_buf.dtype)

        def process_head(h, fetch_during, fetch_after):
            wait_until_filled(kv_buf.at[h % 2], sems.at[h % 2])

            def step(b):
                attend(h, b)
                fetch_during(b)

            _loop(0, B, step)
            if fetch_after is not None:
                _loop(0, B, fetch_after)

        for i, p in enumerate(q_order):
            piece_heads = pl.ds((p % pieces) * heads, heads)
            pltpu.make_async_copy(
                q_hbm.at[p // pieces, piece_heads],
                q_buf.at[p // pieces, piece_heads],
                sems.at[2],
            ).start(priority=i % 2)
        _loop(0, rounds, lambda piece: fetch_head(0, piece))
        _loop(0, B, lambda piece: fetch_head(1, piece))
        wait_until_filled(q_buf, sems.at[2])

        _loop(
            0,
            H - 3,
            lambda h: process_head(
                h,
                lambda i: fetch_head(h + 1, B + i),
                lambda i: fetch_head(h + 2, i),
            ),
        )
        process_head(
            H - 3, lambda i: fetch_head(H - 2, B + i), fetch_first_half
        )
        process_head(H - 2, fetch_second_half, None)

        wait_until_filled(kv_buf.at[last_slot, :, pl.ds(0, half)], sems.at[last_slot])
        _loop(0, half, lambda b: attend(last, b))

        _loop(0, before_final, lambda i: wait_second_half(i, sems.at[1 - last_slot]))
        for i, p in enumerate(out_order):
            b, first_head = p // pieces, (p % pieces) * heads
            pending = b >= half and first_head + heads == H
            start_out(b, first_head, heads - 1 if pending else heads, i % 2)
        _loop(before_final, rounds * half, lambda i: wait_second_half(i, sems.at[2]))

        for b in range(half, B):
            attend(last, b)
        start_out(pl.ds(half, half), last, 1, 0)
        pltpu.make_async_copy(o_buf, o_hbm, sems.at[last_slot]).wait()

    return pl.pallas_call(
        kernel,
        in_specs=[pl.BlockSpec(memory_space=pl.ANY)] * 3,
        out_specs=pl.BlockSpec(memory_space=pl.ANY),
        out_shape=jax.ShapeDtypeStruct(q.shape, q.dtype),
        scratch_shapes=[
            pltpu.VMEM(q.shape, q.dtype),
            pltpu.VMEM((2, 2, B, Sk, D), k.dtype),
            pltpu.VMEM(q.shape, q.dtype),
            pltpu.SemaphoreType.DMA((3,)),
        ],
        compiler_params=pltpu.CompilerParams(vmem_limit_bytes=48 * 1024 * 1024),
    )(q, k, v)
```
